```python
import jax
import jax.numpy as jnp

def _softmax(x, axis=-1):
    return jax.nn.softmax(x, axis=axis)

def _gelu(x):
    return jax.nn.gelu(x, approximate=True)

def _silu(x):
    return jax.nn.silu(x)

def _sigmoid(x):
    return jax.nn.sigmoid(x)

def _layernorm(x, axis=-1, eps=1e-05):
    m = jnp.mean(x, axis=axis, keepdims=True)
    v = jnp.var(x, axis=axis, keepdims=True)
    return (x - m) / jnp.sqrt(v + eps)

def _scatter_add(tgt, idx, src, axis=0):
    return tgt.at[idx].add(src)

def _segment_sum(src, seg, n):
    return jax.ops.segment_sum(src, seg, n)

class _Rng:

    def __init__(self, key):
        self._k = key

    def _next(self):
        self._k, sub = jax.random.split(self._k)
        return sub

    def normal(self, shape):
        return jax.random.normal(self._next(), shape, dtype=jnp.bfloat16)

    def randint(self, lo, hi, shape):
        return jax.random.randint(self._next(), shape, lo, hi, dtype=jnp.int32)

    def uniform(self, shape, lo=0.0, hi=1.0):
        return jax.random.uniform(self._next(), shape, jnp.bfloat16, lo, hi)

    def permutation(self, n):
        return jax.random.permutation(self._next(), n)
kernel_name = 'interleave_layers__linear_kernel_hedgehog__mixer_gmlp__prompt'

def _fwd_setup_inputs():
    _rng = _Rng(jax.random.key(int.from_bytes(__import__("os").urandom(4), "little")))
    _w = lambda a: (lambda t: t.astype(jnp.bfloat16) if jnp.issubdtype(t.dtype, jnp.floating) else t)(jnp.asarray(a))

    def _A_setup():
        B, S, D, H = (1, 2048, 640, 32)
        Dh = D // H
        return {'x': _w((lambda *s: _rng.normal(s) * 0.05)(B, S, D)), 'wqkv': _w((lambda *s: _rng.normal(s) * 0.05)(D, 3 * D)), 'w_phi': _w((lambda *s: _rng.normal(s) * 0.05)(H, Dh, Dh) * Dh ** (-0.5)), 'wo': _w((lambda *s: _rng.normal(s) * 0.05)(D, D))}
    _A_in = _A_setup()

    def _B_setup():
        B, S, D, F = (1, 2048, 640, 1536)
        Fh = F // 2
        return {'x': _w((lambda *s: _rng.normal(s) * 0.05)(B, S, D)), 'w_in': _w((lambda *s: _rng.normal(s) * 0.05)(D, 2 * Fh)), 'w_sp': _w(0.01 * (lambda *s: _rng.normal(s) * 0.05)(S, S)), 'b_sp': _w(1.0 + 0.01 * (lambda *s: _rng.normal(s) * 0.05)(S)), 'w_out': _w((lambda *s: _rng.normal(s) * 0.05)(Fh, D))}
    _B_in = _B_setup()
    return {'A_x': _A_in['x'], 'A_wqkv': _A_in['wqkv'], 'A_w_phi': _A_in['w_phi'], 'A_wo': _A_in['wo'], 'B_x': _B_in['x'], 'B_w_in': _B_in['w_in'], 'B_w_sp': _B_in['w_sp'], 'B_b_sp': _B_in['b_sp'], 'B_w_out': _B_in['w_out']}

def _fwd_reference(A_x, A_wqkv, A_w_phi, A_wo, B_x, B_w_in, B_w_sp, B_b_sp, B_w_out):

    def _A_ref(x, wqkv, w_phi, wo):
        B, S, D = x.shape
        H = 32
        Dh = D // H
        qkv = (lambda x, *d: x.transpose(*d))((x @ wqkv).reshape(B, S, 3, H, Dh), 2, 0, 3, 1, 4)
        q, k, v = (qkv[0], qkv[1], qkv[2])
        pq = jnp.einsum('bhsd,hdf->bhsf', q, w_phi)
        pk = jnp.einsum('bhsd,hdf->bhsf', k, w_phi)
        phi_q = jnp.concatenate([_softmax(pq, axis=-1), _softmax(-pq, axis=-1)], axis=-1)
        phi_k = jnp.concatenate([_softmax(pk, axis=-1), _softmax(-pk, axis=-1)], axis=-1)
        kv = jnp.einsum('bhsf,bhsd->bhfd', phi_k, v)
        z = jnp.einsum('bhsf->bhf', phi_k)
        num = jnp.einsum('bhqf,bhfd->bhqd', phi_q, kv)
        den = jnp.einsum('bhqf,bhf->bhq', phi_q, z)[..., None] + 1e-06
        o = num / den
        return (lambda x, *d: x.transpose(*d))(o, 0, 2, 1, 3).reshape(B, S, D) @ wo

    def _B_ref(x, w_in, w_sp, b_sp, w_out):
        B, S, D = x.shape
        F = w_in.shape[-1]
        Fh = F // 2
        z = _gelu(jnp.einsum('bsd,df->bsf', x, w_in))
        z1 = z[..., :Fh].copy()
        z2 = _layernorm(z[..., Fh:], axis=-1)
        g = jnp.einsum('ts,bsf->btf', w_sp, z2) + b_sp[None, :, None]
        return jnp.einsum('bsf,fd->bsd', z1 * g, w_out)
    x = A_x
    x = x + _A_ref(_layernorm(x, axis=-1), A_wqkv, A_w_phi, A_wo)
    x = x + _B_ref(_layernorm(x, axis=-1), B_w_in, B_w_sp, B_b_sp, B_w_out)
    x = x + _A_ref(_layernorm(x, axis=-1), A_wqkv, A_w_phi, A_wo)
    x = x + _B_ref(_layernorm(x, axis=-1), B_w_in, B_w_sp, B_b_sp, B_w_out)
    return x

def setup_inputs():
    _inp = _fwd_setup_inputs()
    _gk = jax.random.fold_in(jax.random.key(int.from_bytes(__import__("os").urandom(4), "little")), 2 ** 31 - 1)
    _shapes = [[1, 2048, 640]]
    _dtypes = ['bfloat16']
    _gks = jax.random.split(_gk, len(_shapes))
    _gs = [jax.random.normal(k, s, dtype=jnp.dtype(d)) * 0.05 for k, s, d in zip(_gks, _shapes, _dtypes)]
    _inp['grad_out'] = _gs[0]
    return _inp

def reference(A_x, A_wqkv, A_w_phi, A_wo, B_w_in, B_w_sp, B_b_sp, B_w_out, B_x, grad_out):
    _const = dict(B_x=B_x)

    def _f(*_d):
        return _fwd_reference(**{'A_x': _d[0], 'A_wqkv': _d[1], 'A_w_phi': _d[2], 'A_wo': _d[3], 'B_w_in': _d[4], 'B_w_sp': _d[5], 'B_b_sp': _d[6], 'B_w_out': _d[7], **_const})
    _out, _vjp = jax.vjp(_f, A_x, A_wqkv, A_w_phi, A_wo, B_w_in, B_w_sp, B_b_sp, B_w_out)
    _grads = _vjp(grad_out)
    _out0 = jnp.asarray(_out)
    return (_out0, *[jnp.asarray(_g) for _g in _grads])
```

```python
import jax
import jax.numpy as jnp
from jax import lax
import jax.experimental.pallas as pl
import jax.experimental.pallas.tpu as pltpu

F32 = jnp.float32
BF = jnp.bfloat16
TB = 512


def _nn(a, b):
    return jnp.dot(a, b, preferred_element_type=F32)


def _nt(a, b):
    return lax.dot_general(a, b, (((1,), (1,)), ((), ())), preferred_element_type=F32)


def _tn(a, b):
    return lax.dot_general(a, b, (((0,), (0,)), ((), ())), preferred_element_type=F32)


def _ln(x):
    n = x.shape[0]
    m = jnp.sum(x, axis=0, keepdims=True) * (1.0 / n)
    xc = x - m
    v = jnp.sum(xc * xc, axis=0, keepdims=True) * (1.0 / n)
    r = lax.rsqrt(v + 1e-5)
    return xc * r, r


def _ln_bwd(dy, y, r):
    n = dy.shape[0]
    a = jnp.sum(dy, axis=0, keepdims=True) * (1.0 / n)
    b = jnp.sum(dy * y, axis=0, keepdims=True) * (1.0 / n)
    return r * (dy - a - y * b)


_GC = 0.7978845608028654
_GA = 0.044715


def _gelu(u):
    t = jnp.tanh(_GC * (u + _GA * (u * u * u)))
    return 0.5 * u * (1.0 + t)


def _gelu_and_grad(u):
    u2 = u * u
    t = jnp.tanh(_GC * (u + _GA * (u2 * u)))
    h = 0.5 * (1.0 + t)
    gr = h + 0.5 * u * (1.0 - t * t) * (_GC * (1.0 + 3.0 * _GA * u2))
    return u * h, gr


def _lanes(v, n):
    return jnp.concatenate([v] * n, axis=1) if n > 1 else v


def _lane_partial(v):
    acc = v[:, 0:128]
    for j in range(1, v.shape[1] // 128):
        acc = acc + v[:, j * 128:(j + 1) * 128]
    return acc


def _pm_softmax(p, dh):
    t = p.shape[1]
    p3 = p.reshape(dh, 8, t)
    mx = jnp.max(p3, axis=0, keepdims=True)
    mn = jnp.min(p3, axis=0, keepdims=True)
    ep = jnp.exp(p3 - mx)
    en = jnp.exp(mn - p3)
    sp = 1.0 / jnp.sum(ep, axis=0, keepdims=True)
    sn = 1.0 / jnp.sum(en, axis=0, keepdims=True)
    return (ep * sp).reshape(dh * 8, t), (en * sn).reshape(dh * 8, t)


def _pm_softmax_bwd(phi, dphi, dh):
    t = phi.shape[1]
    gw = dh * 8
    pp = phi[0:gw].reshape(dh, 8, t)
    pn = phi[gw:2 * gw].reshape(dh, 8, t)
    dp = dphi[0:gw].reshape(dh, 8, t)
    dn = dphi[gw:2 * gw].reshape(dh, 8, t)
    a = jnp.sum(pp * dp, axis=0, keepdims=True)
    b = jnp.sum(pn * dn, axis=0, keepdims=True)
    return (pp * (dp - a) - pn * (dn - b)).reshape(gw, t)


def _kernel(x_h, wqkv_h, wphi_ref, wo_h, win_h, wsp_h, bsp_ref, wout_h, gout_h,
            out_h, dx_h, dwqkv_h, dwphi_ref, dwo_h, dwin_h, dwsp_h, dbsp_ref, dwout_h,
            wn, wt, wrt, wo, wot, win, wint, wout, woutt, wsp,
            xt, yt, rs, phiq, phik, vt, ot, rden, ut, z2t, gt, dgt, dgn,
            gacc, dwoacc, dwinacc, dwoutacc, dbacc,
            kvacc, kvt, dkvt, zacc, zb, mt, w2, sems):
    S = xt.shape[1]
    D = xt.shape[0]
    H, DH = wphi_ref.shape[0], wphi_ref.shape[1]
    FH = z2t.shape[1]
    NG = H // 8
    GW = DH * 8
    PW = 2 * GW
    NB = S // TB
    NL = TB // 128

    def blk(i):
        return pl.ds(pl.multiple_of(i * TB, TB), TB)

    cx = pltpu.make_async_copy(x_h, dgn.at[:, pl.ds(0, D)], sems.at[0])
    cq = pltpu.make_async_copy(wqkv_h, wn, sems.at[1])
    co = pltpu.make_async_copy(wo_h, wo, sems.at[2])
    ci = pltpu.make_async_copy(win_h, win, sems.at[3])
    cs = pltpu.make_async_copy(wsp_h, wsp, sems.at[4])
    cw = pltpu.make_async_copy(wout_h, wout, sems.at[5])
    cg = pltpu.make_async_copy(gout_h, dgn.at[:, pl.ds(FH, D)], sems.at[6])
    cq.start()
    cx.start()
    co.start()
    ci.start()
    cw.start()
    cs.start()
    cg.start()

    for h in range(H):
        w2[h * DH:(h + 1) * DH, :] = wphi_ref[h].astype(F32)
    ci_ = lax.broadcasted_iota(jnp.int32, (GW, GW), 0)
    ri_ = lax.broadcasted_iota(jnp.int32, (GW, GW), 1)
    lo = (ci_ & 7) * DH
    hmask_t = jnp.logical_and(ri_ >= lo, ri_ < lo + DH)
    selt = ((lax.broadcasted_iota(jnp.int32, (GW, DH), 0) >> 3)
            == lax.broadcasted_iota(jnp.int32, (GW, DH), 1)).astype(F32).astype(BF)
    for g in range(NG):
        m = _nt(selt, w2[g * GW:(g + 1) * GW, :].astype(BF))
        mt[g] = jnp.where(hmask_t, m, 0.0).astype(BF)

    gacc[...] = jnp.zeros_like(gacc)
    dwoacc[...] = jnp.zeros_like(dwoacc)
    dwinacc[...] = jnp.zeros_like(dwinacc)
    dwoutacc[...] = jnp.zeros_like(dwoutacc)
    dbacc[...] = jnp.zeros_like(dbacc)

    cq.wait()
    wrt[...] = wn[:, 0:2 * D].T
    wt[2 * D:3 * D, :] = wn[:, 2 * D:3 * D].T
    for j in range(2 * NG):
        wt[j * GW:(j + 1) * GW, :] = _nn(mt[j % NG], wrt[j * GW:(j + 1) * GW, :]).astype(BF)
    wn[:, 0:2 * D] = wt[0:2 * D, :].T
    cx.wait()

    def xin(i, c):
        xt[:, blk(i)] = dgn[blk(i), 0:D].T.astype(F32)
        return c
    lax.fori_loop(0, NB, xin, 0)
    co.wait()
    wot[...] = wo[...].T
    ci.wait()
    wint[...] = win[...].T
    cw.wait()
    woutt[...] = wout[...].T
    cs.wait()

    vr = lax.broadcasted_iota(jnp.int32, (GW, PW), 0)
    vlo = (lax.broadcasted_iota(jnp.int32, (GW, PW), 1) & 7) * DH
    kvmask = jnp.logical_and(vr >= vlo, vr < vlo + DH)

    def fwd_layer(l, c):
        kvacc[...] = jnp.zeros_like(kvacc)
        zacc[...] = jnp.zeros_like(zacc)

        def a1(i, c):
            b = blk(i)
            y, r = _ln(xt[:, b])
            yb = y.astype(BF)
            yt[2 * l, :, b] = yb
            rs[2 * l, :, b] = r
            vb = _nn(wt[2 * D:3 * D, :], yb).astype(BF)
            vt[l, :, b] = vb
            for g in range(NG):
                sp, sn = _pm_softmax(_nn(wt[D + g * GW:D + (g + 1) * GW, :], yb), DH)
                zacc[g * PW:g * PW + GW, :] += _lane_partial(sp)
                zacc[g * PW + GW:(g + 1) * PW, :] += _lane_partial(sn)
                pk = jnp.concatenate([sp.astype(BF), sn.astype(BF)], axis=0)
                phik[l, g * PW:(g + 1) * PW, b] = pk
                kvacc[g * GW:(g + 1) * GW, :] += _nt(vb[g * GW:(g + 1) * GW], pk)
            for g in range(NG):
                sp, sn = _pm_softmax(_nn(wt[g * GW:(g + 1) * GW, :], yb), DH)
                phiq[l, g * PW:g * PW + GW, b] = sp.astype(BF)
                phiq[l, g * PW + GW:(g + 1) * PW, b] = sn.astype(BF)
            return c
        lax.fori_loop(0, NB, a1, 0)

        for g in range(NG):
            kvt[l, g * GW:(g + 1) * GW, :] = jnp.where(
                kvmask, kvacc[g * GW:(g + 1) * GW, :], 0.0).astype(BF)
        zb[l] = jnp.broadcast_to(jnp.sum(zacc[...], axis=1, keepdims=True), zacc.shape)

        def a2b1(i, c):
            b = blk(i)
            os_ = []
            for g in range(NG):
                ph = phiq[l, g * PW:(g + 1) * PW, b].astype(F32).reshape(2 * DH, 8, TB)
                z = _lanes(zb[l, g * PW:(g + 1) * PW, :], NL).reshape(2 * DH, 8, TB)
                rd = 1.0 / (jnp.sum(ph * z, axis=0) + 1e-6)
                rden[l, g * 8:(g + 1) * 8, b] = rd
                psi = (ph * rd[None]).reshape(PW, TB).astype(BF)
                phiq[l, g * PW:(g + 1) * PW, b] = psi
                os_.append(_nn(kvt[l, g * GW:(g + 1) * GW, :], psi).astype(BF))
            ob = jnp.concatenate(os_, axis=0)
            ot[l, :, b] = ob
            x = xt[:, b] + _nn(wot[...], ob)
            xt[:, b] = x
            y, r = _ln(x)
            yb = y.astype(BF)
            yt[2 * l + 1, :, b] = yb
            rs[2 * l + 1, :, b] = r
            u2 = _nn(wint[FH:2 * FH, :], yb)
            ut[l, FH:2 * FH, b] = u2.astype(BF)
            z2, r2 = _ln(_gelu(u2))
            z2t[l, :, b] = z2.astype(BF)
            rs[4 + l, :, b] = r2
            u1 = _nn(wint[0:FH, :], yb)
            ut[l, 0:FH, b] = u1.astype(BF)
            dgt[:, b] = _gelu(u1).astype(BF)
            return c
        lax.fori_loop(0, NB, a2b1, 0)

        def b2(i, c):
            b = blk(i)
            gv = _nt(z2t[l], wsp[b, :]) + bsp_ref[:, b].astype(F32)
            gt[l, :, b] = gv.astype(BF)
            hb = (dgt[:, b].astype(F32) * gv).astype(BF)
            xt[:, b] += _nn(woutt[...], hb)
            return c
        lax.fori_loop(0, NB, b2, 0)
        return c
    lax.fori_loop(0, 2, fwd_layer, 0)

    cg.wait()

    def xout(i, c):
        b = blk(i)
        dgn[b, 0:D] = xt[:, b].astype(BF).T
        xt[:, b] = dgn[b, FH:FH + D].T.astype(F32)
        return c
    lax.fori_loop(0, NB, xout, 0)
    cout = pltpu.make_async_copy(dgn.at[:, pl.ds(0, D)], out_h, sems.at[0])
    cout.start()

    cdsp = pltpu.make_async_copy(wsp, dwsp_h, sems.at[4])

    def bwd_layer(li, c):
        l = 1 - li

        @pl.when(li == 1)
        def _():
            cout.wait()

        def bb1(i, c):
            b = blk(i)
            dxb = xt[:, b].astype(BF)
            dh = _nn(wout[...], dxb)
            z1, gr = _gelu_and_grad(ut[l, 0:FH, b].astype(F32))
            gv = gt[l, :, b].astype(F32)
            dwoutacc[...] += _nt((z1 * gv).astype(BF), dxb)
            dg = dh * z1
            dbacc[:, b] += jnp.sum(dg, axis=0, keepdims=True)
            dgb = dg.astype(BF)
            dgt[:, b] = dgb
            dgn[b, pl.ds(pl.multiple_of(l * FH, 128), FH)] = dgb.T
            ut[l, 0:FH, b] = (dh * gv * gr).astype(BF)
            return c
        lax.fori_loop(0, NB, bb1, 0)

        def bb2(i, c):
            b = blk(i)
            dz2n = _nn(dgt[...], wsp[:, b])
            dz2 = _ln_bwd(dz2n, z2t[l, :, b].astype(F32), rs[4 + l, :, b])
            _, gr = _gelu_and_grad(ut[l, FH:2 * FH, b].astype(F32))
            du = jnp.concatenate([ut[l, 0:FH, b], (dz2 * gr).astype(BF)], axis=0)
            yb = yt[2 * l + 1, :, b]
            dwinacc[...] += _nt(yb, du)
            dy = _nn(win[...], du)
            xt[:, b] += _ln_bwd(dy, yb.astype(F32), rs[2 * l + 1, :, b])
            return c
        lax.fori_loop(0, NB, bb2, 0)

        @pl.when(li == 1)
        def _():
            RB = 256

            def dsp(i, c):
                r = pl.ds(pl.multiple_of(i * RB, RB), RB)
                wsp[r, :] = (_nn(dgn[r, 0:FH], z2t[0]) + _nn(dgn[r, FH:2 * FH], z2t[1])).astype(BF)
                return c
            lax.fori_loop(0, S // RB, dsp, 0)
            cdsp.start()

        kvacc[...] = jnp.zeros_like(kvacc)
        zacc[...] = jnp.zeros_like(zacc)

        def ab1(i, c):
            b = blk(i)
            dxb = xt[:, b].astype(BF)
            dwoacc[...] += _nt(ot[l, :, b], dxb)
            dob = _nn(wo[...], dxb).astype(BF)
            for g in range(NG):
                dog = dob[g * GW:(g + 1) * GW]
                psib = phiq[l, g * PW:(g + 1) * PW, b]
                kvacc[g * GW:(g + 1) * GW, :] += _nt(dog, psib)
                dpsi = _tn(kvt[l, g * GW:(g + 1) * GW, :], dog).reshape(2 * DH, 8, TB)
                psi = psib.astype(F32).reshape(2 * DH, 8, TB)
                rd = rden[l, g * 8:(g + 1) * 8, b]
                dden = -rd * jnp.sum(dpsi * psi, axis=0)
                ph = psi * (1.0 / rd)[None]
                z = _lanes(zb[l, g * PW:(g + 1) * PW, :], NL).reshape(2 * DH, 8, TB)
                dph = dpsi * rd[None] + dden[None] * z
                zacc[g * PW:(g + 1) * PW, :] += _lane_partial((ph * dden[None]).reshape(PW, TB))
                dp = _pm_softmax_bwd(ph.reshape(PW, TB), dph.reshape(PW, TB), DH)
                ot[l, g * GW:(g + 1) * GW, b] = dp.astype(BF)
            return c
        lax.fori_loop(0, NB, ab1, 0)

        for g in range(NG):
            dkvt[g * GW:(g + 1) * GW, :] = jnp.where(
                kvmask, kvacc[g * GW:(g + 1) * GW, :], 0.0).astype(BF)
        zacc[...] = jnp.broadcast_to(jnp.sum(zacc[...], axis=1, keepdims=True), zacc.shape)

        def ab2(i, c):
            b = blk(i)
            parts = [ot[l, :, b]]
            dvs = []
            for g in range(NG):
                pkb = phik[l, g * PW:(g + 1) * PW, b]
                dk = dkvt[g * GW:(g + 1) * GW, :]
                dph = _tn(dk, vt[l, g * GW:(g + 1) * GW, b]) + _lanes(zacc[g * PW:(g + 1) * PW, :], NL)
                parts.append(_pm_softmax_bwd(pkb.astype(F32), dph, DH).astype(BF))
                dvs.append(_nn(dk, pkb).astype(BF))
            dp = jnp.concatenate(parts + dvs, axis=0)
            yb = yt[2 * l, :, b]
            gacc[...] += _nt(dp, yb)
            dy = _nn(wn[...], dp)
            xt[:, b] += _ln_bwd(dy, yb.astype(F32), rs[2 * l, :, b])
            return c
        lax.fori_loop(0, NB, ab2, 0)
        return c
    lax.fori_loop(0, 2, bwd_layer, 0)

    def dxout(i, c):
        b = blk(i)
        dgn[b, 0:D] = xt[:, b].astype(BF).T
        return c
    lax.fori_loop(0, NB, dxout, 0)
    cdx = pltpu.make_async_copy(dgn.at[:, pl.ds(0, D)], dx_h, sems.at[0])
    cdx.start()
    win[...] = dwinacc[...].astype(BF)
    c3 = pltpu.make_async_copy(win, dwin_h, sems.at[3])
    c3.start()
    wout[...] = dwoutacc[...].astype(BF)
    c5 = pltpu.make_async_copy(wout, dwout_h, sems.at[5])
    c5.start()
    wo[...] = dwoacc[...].astype(BF)
    c2 = pltpu.make_async_copy(wo, dwo_h, sems.at[2])
    c2.start()
    dbsp_ref[...] = dbacc[...].astype(BF)

    sel = ((lax.broadcasted_iota(jnp.int32, (DH, GW), 1) >> 3)
           == lax.broadcasted_iota(jnp.int32, (DH, GW), 0)).astype(F32).astype(BF)
    for g in range(NG):
        dm = jnp.zeros((GW, GW), F32)
        for j in (g, NG + g):
            gb = gacc[j * GW:(j + 1) * GW, :].astype(BF)
            wt[j * GW:(j + 1) * GW, :] = _tn(mt[g], gb).astype(BF)
            dm = dm + _nt(gb, wrt[j * GW:(j + 1) * GW, :])
        w2[g * GW:(g + 1) * GW, :] = _tn(jnp.where(hmask_t, dm, 0.0).astype(BF), selt)
    wt[2 * D:3 * D, :] = gacc[2 * D:3 * D, :].astype(BF)
    wn[...] = wt[...].T
    c1 = pltpu.make_async_copy(wn, dwqkv_h, sems.at[1])
    c1.start()
    for h in range(H):
        dwphi_ref[h] = w2[h * DH:(h + 1) * DH, :].astype(BF)
    del sel
    cdsp.wait()
    cdx.wait()
    c3.wait()
    c5.wait()
    c2.wait()
    c1.wait()


@jax.jit
def pallas_interleave_layers__linear_kernel_hedgehog__mixer_gmlp__prompt_kernel(
    A_x: jax.Array,
    A_wqkv: jax.Array,
    A_w_phi: jax.Array,
    A_wo: jax.Array,
    B_x: jax.Array,
    B_w_in: jax.Array,
    B_w_sp: jax.Array,
    B_b_sp: jax.Array,
    B_w_out: jax.Array,
    grad_out: jax.Array,
):
    del B_x
    _, S, D = A_x.shape
    H, DH, _ = A_w_phi.shape
    F = B_w_in.shape[1]
    FH = F // 2
    any_spec = pl.BlockSpec(memory_space=pl.ANY)
    vm = pl.BlockSpec(memory_space=pltpu.VMEM)
    V = pltpu.VMEM
    scratch = [
        V((D, 3 * D), BF), V((3 * D, D), BF), V((2 * D, D), BF),
        V((D, D), BF), V((D, D), BF),
        V((D, F), BF), V((F, D), BF),
        V((FH, D), BF), V((D, FH), BF),
        V((S, S), BF),
        V((D, S), F32), V((4, D, S), BF), V((6, 1, S), F32),
        V((2, 2 * D, S), BF), V((2, 2 * D, S), BF),
        V((2, D, S), BF), V((2, D, S), BF), V((2, H, S), F32),
        V((2, F, S), BF), V((2, FH, S), BF), V((2, FH, S), BF),
        V((FH, S), BF), V((S, F), BF),
        V((3 * D, D), F32), V((D, D), F32), V((D, F), F32),
        V((FH, D), F32), V((1, S), F32),
        V((D, 16 * DH), F32), V((2, D, 16 * DH), BF), V((D, 16 * DH), BF),
        V((2 * D, 128), F32), V((2, 2 * D, 128), F32),
        V((H // 8, 8 * DH, 8 * DH), BF), V((D, DH), F32),
        pltpu.SemaphoreType.DMA((7,)),
    ]
    sd = jax.ShapeDtypeStruct
    outs = pl.pallas_call(
        _kernel,
        in_specs=[any_spec, any_spec, vm, any_spec, any_spec, any_spec, vm, any_spec, any_spec],
        out_specs=[any_spec, any_spec, any_spec, vm, any_spec, any_spec, any_spec, vm, any_spec],
        out_shape=[sd((S, D), BF), sd((S, D), BF), sd((D, 3 * D), BF), sd((H, DH, DH), BF),
                   sd((D, D), BF), sd((D, F), BF), sd((S, S), BF), sd((1, S), BF), sd((FH, D), BF)],
        scratch_shapes=scratch,
        compiler_params=pltpu.CompilerParams(vmem_limit_bytes=127 * 1024 * 1024),
    )(A_x.reshape(S, D), A_wqkv, A_w_phi, A_wo, B_w_in, B_w_sp, B_b_sp.reshape(1, S), B_w_out,
      grad_out.reshape(S, D))
    out, dx, dwqkv, dwphi, dwo, dwin, dwsp, dbsp, dwout = outs
    return (out.reshape(1, S, D), dx.reshape(1, S, D), dwqkv, dwphi, dwo, dwin, dwsp,
            dbsp.reshape(S), dwout)
```

```python
import jax
import jax.numpy as jnp
from jax import lax
import jax.experimental.pallas as pl
import jax.experimental.pallas.tpu as pltpu

F32 = jnp.float32
BF = jnp.bfloat16
TB = 512


def _nn(a, b):
    return jnp.dot(a, b, preferred_element_type=F32)


def _nt(a, b):
    return lax.dot_general(a, b, (((1,), (1,)), ((), ())), preferred_element_type=F32)


def _tn(a, b):
    return lax.dot_general(a, b, (((0,), (0,)), ((), ())), preferred_element_type=F32)


def _ln(x):
    n = x.shape[0]
    m = jnp.sum(x, axis=0, keepdims=True) * (1.0 / n)
    xc = x - m
    v = jnp.sum(xc * xc, axis=0, keepdims=True) * (1.0 / n)
    r = lax.rsqrt(v + 1e-5)
    return xc * r, r


def _ln_bwd(dy, y, r):
    n = dy.shape[0]
    a = jnp.sum(dy, axis=0, keepdims=True) * (1.0 / n)
    b = jnp.sum(dy * y, axis=0, keepdims=True) * (1.0 / n)
    return r * (dy - a - y * b)


_GC = 0.7978845608028654
_GA = 0.044715


def _gelu(u):
    t = jnp.tanh(_GC * (u + _GA * (u * u * u)))
    return 0.5 * u * (1.0 + t)


def _gelu_and_grad(u):
    u2 = u * u
    t = jnp.tanh(_GC * (u + _GA * (u2 * u)))
    h = 0.5 * (1.0 + t)
    gr = h + 0.5 * u * (1.0 - t * t) * (_GC * (1.0 + 3.0 * _GA * u2))
    return u * h, gr


def _lanes(v, n):
    return jnp.concatenate([v] * n, axis=1) if n > 1 else v


def _lane_partial(v):
    acc = v[:, 0:128]
    for j in range(1, v.shape[1] // 128):
        acc = acc + v[:, j * 128:(j + 1) * 128]
    return acc


def _pm_softmax(p, dh):
    t = p.shape[1]
    p3 = p.reshape(dh, 8, t)
    mx = jnp.max(p3, axis=0, keepdims=True)
    mn = jnp.min(p3, axis=0, keepdims=True)
    ep = jnp.exp(p3 - mx)
    en = jnp.exp(mn - p3)
    sp = 1.0 / jnp.sum(ep, axis=0, keepdims=True)
    sn = 1.0 / jnp.sum(en, axis=0, keepdims=True)
    return (ep * sp).reshape(dh * 8, t), (en * sn).reshape(dh * 8, t)


def _pm_softmax_bwd(phi, dphi, dh):
    t = phi.shape[1]
    gw = dh * 8
    pp = phi[0:gw].reshape(dh, 8, t)
    pn = phi[gw:2 * gw].reshape(dh, 8, t)
    dp = dphi[0:gw].reshape(dh, 8, t)
    dn = dphi[gw:2 * gw].reshape(dh, 8, t)
    a = jnp.sum(pp * dp, axis=0, keepdims=True)
    b = jnp.sum(pn * dn, axis=0, keepdims=True)
    return (pp * (dp - a) - pn * (dn - b)).reshape(gw, t)


def _kernel(x_h, wqkv_h, wphi_ref, wo_h, win_h, wsp_h, bsp_ref, wout_h, gout_h,
            out_h, dx_h, dwqkv_h, dwphi_ref, dwo_h, dwin_h, dwsp_h, dbsp_ref, dwout_h,
            wn, wt, wrt, wo, wot, win, wint, wout, woutt, wsp,
            xt, yt, rs, phiq, phik, vt, ot, rden, ut, z2t, gt, dgt, dgn,
            gacc, dwoacc, dwinacc, dwoutacc, dbacc,
            kvacc, kvt, dkvt, zacc, zb, mt, w2, sems):
    S = xt.shape[1]
    D = xt.shape[0]
    H, DH = wphi_ref.shape[0], wphi_ref.shape[1]
    FH = z2t.shape[1]
    NG = H // 8
    GW = DH * 8
    PW = 2 * GW
    NB = S // TB
    NL = TB // 128

    def blk(i):
        return pl.ds(pl.multiple_of(i * TB, TB), TB)

    cx = pltpu.make_async_copy(x_h, dgn.at[:, pl.ds(0, D)], sems.at[0])
    cq = pltpu.make_async_copy(wqkv_h, wn, sems.at[1])
    co = pltpu.make_async_copy(wo_h, wo, sems.at[2])
    ci = pltpu.make_async_copy(win_h, win, sems.at[3])
    cs = pltpu.make_async_copy(wsp_h, wsp, sems.at[4])
    cw = pltpu.make_async_copy(wout_h, wout, sems.at[5])
    cg = pltpu.make_async_copy(gout_h, dgn.at[:, pl.ds(FH, D)], sems.at[6])
    cq.start()
    cx.start()

    for h in range(H):
        w2[h * DH:(h + 1) * DH, :] = wphi_ref[h].astype(F32)
    ci_ = lax.broadcasted_iota(jnp.int32, (GW, GW), 0)
    ri_ = lax.broadcasted_iota(jnp.int32, (GW, GW), 1)
    lo = (ci_ & 7) * DH
    hmask_t = jnp.logical_and(ri_ >= lo, ri_ < lo + DH)
    selt = ((lax.broadcasted_iota(jnp.int32, (GW, DH), 0) >> 3)
            == lax.broadcasted_iota(jnp.int32, (GW, DH), 1)).astype(F32).astype(BF)
    for g in range(NG):
        m = _nt(selt, w2[g * GW:(g + 1) * GW, :].astype(BF))
        mt[g] = jnp.where(hmask_t, m, 0.0).astype(BF)

    gacc[...] = jnp.zeros_like(gacc)
    dwoacc[...] = jnp.zeros_like(dwoacc)
    dwinacc[...] = jnp.zeros_like(dwinacc)
    dwoutacc[...] = jnp.zeros_like(dwoutacc)
    dbacc[...] = jnp.zeros_like(dbacc)

    cq.wait()
    wrt[...] = wn[:, 0:2 * D].T
    wt[2 * D:3 * D, :] = wn[:, 2 * D:3 * D].T
    for j in range(2 * NG):
        wt[j * GW:(j + 1) * GW, :] = _nn(mt[j % NG], wrt[j * GW:(j + 1) * GW, :]).astype(BF)
    wn[:, 0:2 * D] = wt[0:2 * D, :].T
    cx.wait()
    co.start()
    ci.start()
    cw.start()
    cs.start()
    cg.start()

    def xin(i, c):
        xt[:, blk(i)] = dgn[blk(i), 0:D].T.astype(F32)
        return c
    lax.fori_loop(0, NB, xin, 0)

    vr = lax.broadcasted_iota(jnp.int32, (GW, PW), 0)
    vlo = (lax.broadcasted_iota(jnp.int32, (GW, PW), 1) & 7) * DH
    kvmask = jnp.logical_and(vr >= vlo, vr < vlo + DH)

    def fwd_layer(l, c):
        kvacc[...] = jnp.zeros_like(kvacc)
        zacc[...] = jnp.zeros_like(zacc)

        def a1(i, c):
            b = blk(i)
            y, r = _ln(xt[:, b])
            yb = y.astype(BF)
            yt[2 * l, :, b] = yb
            rs[2 * l, :, b] = r
            pks = [_nn(wt[D + g * GW:D + (g + 1) * GW, :], yb) for g in range(NG)]
            vb = _nn(wt[2 * D:3 * D, :], yb).astype(BF)
            pqs = [_nn(wt[g * GW:(g + 1) * GW, :], yb) for g in range(NG)]
            vt[l, :, b] = vb
            for g in range(NG):
                sp, sn = _pm_softmax(pks[g], DH)
                zacc[g * PW:g * PW + GW, :] += _lane_partial(sp)
                zacc[g * PW + GW:(g + 1) * PW, :] += _lane_partial(sn)
                pk = jnp.concatenate([sp.astype(BF), sn.astype(BF)], axis=0)
                phik[l, g * PW:(g + 1) * PW, b] = pk
                kvacc[g * GW:(g + 1) * GW, :] += _nt(vb[g * GW:(g + 1) * GW], pk)
            for g in range(NG):
                sp, sn = _pm_softmax(pqs[g], DH)
                phiq[l, g * PW:g * PW + GW, b] = sp.astype(BF)
                phiq[l, g * PW + GW:(g + 1) * PW, b] = sn.astype(BF)
            return c
        lax.fori_loop(0, NB, a1, 0)

        for g in range(NG):
            kvt[l, g * GW:(g + 1) * GW, :] = jnp.where(
                kvmask, kvacc[g * GW:(g + 1) * GW, :], 0.0).astype(BF)
        @pl.when(l == 0)
        def _():
            co.wait()
            wot[...] = wo[...].T
            ci.wait()
            wint[...] = win[...].T
            cw.wait()
            woutt[...] = wout[...].T
            cs.wait()

        zb[l] = jnp.broadcast_to(jnp.sum(zacc[...], axis=1, keepdims=True), zacc.shape)

        def a2b1(i, c):
            b = blk(i)
            os_ = []
            for g in range(NG):
                ph = phiq[l, g * PW:(g + 1) * PW, b].astype(F32).reshape(2 * DH, 8, TB)
                z = _lanes(zb[l, g * PW:(g + 1) * PW, :], NL).reshape(2 * DH, 8, TB)
                rd = 1.0 / (jnp.sum(ph * z, axis=0) + 1e-6)
                rden[l, g * 8:(g + 1) * 8, b] = rd
                psi = (ph * rd[None]).reshape(PW, TB).astype(BF)
                phiq[l, g * PW:(g + 1) * PW, b] = psi
                os_.append(_nn(kvt[l, g * GW:(g + 1) * GW, :], psi).astype(BF))
            ob = jnp.concatenate(os_, axis=0)
            ot[l, :, b] = ob
            x = xt[:, b] + _nn(wot[...], ob)
            xt[:, b] = x
            y, r = _ln(x)
            yb = y.astype(BF)
            yt[2 * l + 1, :, b] = yb
            rs[2 * l + 1, :, b] = r
            u2 = _nn(wint[FH:2 * FH, :], yb)
            ut[l, FH:2 * FH, b] = u2.astype(BF)
            z2, r2 = _ln(_gelu(u2))
            z2t[l, :, b] = z2.astype(BF)
            rs[4 + l, :, b] = r2
            u1 = _nn(wint[0:FH, :], yb)
            ut[l, 0:FH, b] = u1.astype(BF)
            dgt[:, b] = _gelu(u1).astype(BF)
            return c
        lax.fori_loop(0, NB, a2b1, 0)

        def b2(i, c):
            b = blk(i)
            gv = _nt(z2t[l], wsp[b, :]) + bsp_ref[:, b].astype(F32)
            gt[l, :, b] = gv.astype(BF)
            hb = (dgt[:, b].astype(F32) * gv).astype(BF)
            xt[:, b] += _nn(woutt[...], hb)
            return c
        lax.fori_loop(0, NB, b2, 0)
        return c
    lax.fori_loop(0, 2, fwd_layer, 0)

    cg.wait()

    def xout(i, c):
        b = blk(i)
        dgn[b, 0:D] = xt[:, b].astype(BF).T
        xt[:, b] = dgn[b, FH:FH + D].T.astype(F32)
        return c
    lax.fori_loop(0, NB, xout, 0)
    cout = pltpu.make_async_copy(dgn.at[:, pl.ds(0, D)], out_h, sems.at[0])
    cout.start()

    cdsp = pltpu.make_async_copy(wsp, dwsp_h, sems.at[4])
    c3 = pltpu.make_async_copy(win, dwin_h, sems.at[3])
    c5 = pltpu.make_async_copy(wout, dwout_h, sems.at[5])
    c2 = pltpu.make_async_copy(wo, dwo_h, sems.at[2])

    def bwd_layer(li, c):
        l = 1 - li

        @pl.when(li == 1)
        def _():
            cout.wait()

        def bb1(i, c):
            b = blk(i)
            dxb = xt[:, b].astype(BF)
            dh = _nn(wout[...], dxb)
            z1, gr = _gelu_and_grad(ut[l, 0:FH, b].astype(F32))
            gv = gt[l, :, b].astype(F32)
            dwoutacc[...] += _nt((z1 * gv).astype(BF), dxb)
            dg = dh * z1
            dbacc[:, b] += jnp.sum(dg, axis=0, keepdims=True)
            dgb = dg.astype(BF)
            dgt[:, b] = dgb
            dgn[b, pl.ds(pl.multiple_of(l * FH, 128), FH)] = dgb.T
            ut[l, 0:FH, b] = (dh * gv * gr).astype(BF)
            return c
        lax.fori_loop(0, NB, bb1, 0)

        def bb2(i, c):
            b = blk(i)
            dz2n = _nn(dgt[...], wsp[:, b])
            dz2 = _ln_bwd(dz2n, z2t[l, :, b].astype(F32), rs[4 + l, :, b])
            _, gr = _gelu_and_grad(ut[l, FH:2 * FH, b].astype(F32))
            yb = yt[2 * l + 1, :, b]
            du1 = ut[l, 0:FH, b]
            dy = _nn(win[:, 0:FH], du1)
            du2 = (dz2 * gr).astype(BF)
            dy = dy + _nn(win[:, FH:2 * FH], du2)
            dwinacc[:, 0:FH] += _nt(yb, du1)
            dwinacc[:, FH:2 * FH] += _nt(yb, du2)
            xt[:, b] += _ln_bwd(dy, yb.astype(F32), rs[2 * l + 1, :, b])
            return c
        lax.fori_loop(0, NB, bb2, 0)

        @pl.when(li == 1)
        def _():
            win[...] = dwinacc[...].astype(BF)
            c3.start()
            wout[...] = dwoutacc[...].astype(BF)
            c5.start()
            RB = 256

            def dsp(i, c):
                r = pl.ds(pl.multiple_of(i * RB, RB), RB)
                wsp[r, :] = (_nn(dgn[r, 0:FH], z2t[0]) + _nn(dgn[r, FH:2 * FH], z2t[1])).astype(BF)
                return c
            lax.fori_loop(0, S // RB, dsp, 0)
            cdsp.start()

        kvacc[...] = jnp.zeros_like(kvacc)
        zacc[...] = jnp.zeros_like(zacc)

        def ab1(i, c):
            b = blk(i)
            dxb = xt[:, b].astype(BF)
            dob = _nn(wo[...], dxb).astype(BF)
            dpsis = [_tn(kvt[l, g * GW:(g + 1) * GW, :], dob[g * GW:(g + 1) * GW]) for g in range(NG)]
            dwoacc[...] += _nt(ot[l, :, b], dxb)
            for g in range(NG):
                dog = dob[g * GW:(g + 1) * GW]
                psib = phiq[l, g * PW:(g + 1) * PW, b]
                kvacc[g * GW:(g + 1) * GW, :] += _nt(dog, psib)
                dpsi = dpsis[g].reshape(2 * DH, 8, TB)
                psi = psib.astype(F32).reshape(2 * DH, 8, TB)
                rd = rden[l, g * 8:(g + 1) * 8, b]
                dden = -rd * jnp.sum(dpsi * psi, axis=0)
                ph = psi * (1.0 / rd)[None]
                z = _lanes(zb[l, g * PW:(g + 1) * PW, :], NL).reshape(2 * DH, 8, TB)
                dph = dpsi * rd[None] + dden[None] * z
                zacc[g * PW:(g + 1) * PW, :] += _lane_partial((ph * dden[None]).reshape(PW, TB))
                dp = _pm_softmax_bwd(ph.reshape(PW, TB), dph.reshape(PW, TB), DH)
                ot[l, g * GW:(g + 1) * GW, b] = dp.astype(BF)
            return c
        lax.fori_loop(0, NB, ab1, 0)

        for g in range(NG):
            dkvt[g * GW:(g + 1) * GW, :] = jnp.where(
                kvmask, kvacc[g * GW:(g + 1) * GW, :], 0.0).astype(BF)
        @pl.when(li == 1)
        def _():
            wo[...] = dwoacc[...].astype(BF)
            c2.start()

        zacc[...] = jnp.broadcast_to(jnp.sum(zacc[...], axis=1, keepdims=True), zacc.shape)

        def ab2(i, c):
            b = blk(i)
            parts = [ot[l, :, b]]
            dvs = []
            for g in range(NG):
                pkb = phik[l, g * PW:(g + 1) * PW, b]
                dk = dkvt[g * GW:(g + 1) * GW, :]
                dph = _tn(dk, vt[l, g * GW:(g + 1) * GW, b]) + _lanes(zacc[g * PW:(g + 1) * PW, :], NL)
                parts.append(_pm_softmax_bwd(pkb.astype(F32), dph, DH).astype(BF))
                dvs.append(_nn(dk, pkb).astype(BF))
            dp = jnp.concatenate(parts + dvs, axis=0)
            yb = yt[2 * l, :, b]
            dy = _nn(wn[...], dp)
            gacc[...] += _nt(dp, yb)
            xt[:, b] += _ln_bwd(dy, yb.astype(F32), rs[2 * l, :, b])
            return c
        lax.fori_loop(0, NB, ab2, 0)
        return c
    lax.fori_loop(0, 2, bwd_layer, 0)

    def dxout(i, c):
        b = blk(i)
        dgn[b, 0:D] = xt[:, b].astype(BF).T
        return c
    lax.fori_loop(0, NB, dxout, 0)
    cdx = pltpu.make_async_copy(dgn.at[:, pl.ds(0, D)], dx_h, sems.at[0])
    cdx.start()
    dbsp_ref[...] = dbacc[...].astype(BF)

    for g in range(NG):
        dm = jnp.zeros((GW, GW), F32)
        for j in (g, NG + g):
            gb = gacc[j * GW:(j + 1) * GW, :].astype(BF)
            wt[j * GW:(j + 1) * GW, :] = _tn(mt[g], gb).astype(BF)
            dm = dm + _nt(gb, wrt[j * GW:(j + 1) * GW, :])
        w2[g * GW:(g + 1) * GW, :] = _tn(jnp.where(hmask_t, dm, 0.0).astype(BF), selt)
    wt[2 * D:3 * D, :] = gacc[2 * D:3 * D, :].astype(BF)
    wn[...] = wt[...].T
    c1 = pltpu.make_async_copy(wn, dwqkv_h, sems.at[1])
    c1.start()
    for h in range(H):
        dwphi_ref[h] = w2[h * DH:(h + 1) * DH, :].astype(BF)
    cdsp.wait()
    cdx.wait()
    c3.wait()
    c5.wait()
    c2.wait()
    c1.wait()


@jax.jit
def pallas_interleave_layers__linear_kernel_hedgehog__mixer_gmlp__prompt_kernel(
    A_x: jax.Array,
    A_wqkv: jax.Array,
    A_w_phi: jax.Array,
    A_wo: jax.Array,
    B_x: jax.Array,
    B_w_in: jax.Array,
    B_w_sp: jax.Array,
    B_b_sp: jax.Array,
    B_w_out: jax.Array,
    grad_out: jax.Array,
):
    del B_x
    _, S, D = A_x.shape
    H, DH, _ = A_w_phi.shape
    F = B_w_in.shape[1]
    FH = F // 2
    any_spec = pl.BlockSpec(memory_space=pl.ANY)
    vm = pl.BlockSpec(memory_space=pltpu.VMEM)
    V = pltpu.VMEM
    scratch = [
        V((D, 3 * D), BF), V((3 * D, D), BF), V((2 * D, D), BF),
        V((D, D), BF), V((D, D), BF),
        V((D, F), BF), V((F, D), BF),
        V((FH, D), BF), V((D, FH), BF),
        V((S, S), BF),
        V((D, S), F32), V((4, D, S), BF), V((6, 1, S), F32),
        V((2, 2 * D, S), BF), V((2, 2 * D, S), BF),
        V((2, D, S), BF), V((2, D, S), BF), V((2, H, S), F32),
        V((2, F, S), BF), V((2, FH, S), BF), V((2, FH, S), BF),
        V((FH, S), BF), V((S, F), BF),
        V((3 * D, D), F32), V((D, D), F32), V((D, F), F32),
        V((FH, D), F32), V((1, S), F32),
        V((D, 16 * DH), F32), V((2, D, 16 * DH), BF), V((D, 16 * DH), BF),
        V((2 * D, 128), F32), V((2, 2 * D, 128), F32),
        V((H // 8, 8 * DH, 8 * DH), BF), V((D, DH), F32),
        pltpu.SemaphoreType.DMA((7,)),
    ]
    sd = jax.ShapeDtypeStruct
    outs = pl.pallas_call(
        _kernel,
        in_specs=[any_spec, any_spec, vm, any_spec, any_spec, any_spec, vm, any_spec, any_spec],
        out_specs=[any_spec, any_spec, any_spec, vm, any_spec, any_spec, any_spec, vm, any_spec],
        out_shape=[sd((S, D), BF), sd((S, D), BF), sd((D, 3 * D), BF), sd((H, DH, DH), BF),
                   sd((D, D), BF), sd((D, F), BF), sd((S, S), BF), sd((1, S), BF), sd((FH, D), BF)],
        scratch_shapes=scratch,
        compiler_params=pltpu.CompilerParams(vmem_limit_bytes=127 * 1024 * 1024),
    )(A_x.reshape(S, D), A_wqkv, A_w_phi, A_wo, B_w_in, B_w_sp, B_b_sp.reshape(1, S), B_w_out,
      grad_out.reshape(S, D))
    out, dx, dwqkv, dwphi, dwo, dwin, dwsp, dbsp, dwout = outs
    return (out.reshape(1, S, D), dx.reshape(1, S, D), dwqkv, dwphi, dwo, dwin, dwsp,
            dbsp.reshape(S), dwout)
```
